```python
import jax
import jax.numpy as jnp

def _softmax(x, axis=-1):
    return jax.nn.softmax(x, axis=axis)
def _gelu(x):
    return jax.nn.gelu(x, approximate=True)
def _silu(x):
    return jax.nn.silu(x)
def _sigmoid(x):
    return jax.nn.sigmoid(x)
def _layernorm(x, axis=-1, eps=1e-5):
    m = jnp.mean(x, axis=axis, keepdims=True)
    v = jnp.var(x, axis=axis, keepdims=True)
    return (x - m) / jnp.sqrt(v + eps)
def _scatter_add(tgt, idx, src, axis=0):
    return tgt.at[idx].add(src)
def _segment_sum(src, seg, n):
    return jax.ops.segment_sum(src, seg, n)
class _Rng:
    def __init__(self, key):
        self._k = key
    def _next(self):
        self._k, sub = jax.random.split(self._k)
        return sub
    def normal(self, shape):
        return jax.random.normal(self._next(), shape, dtype=jnp.bfloat16)
    def randint(self, lo, hi, shape):
        return jax.random.randint(self._next(), shape, lo, hi, dtype=jnp.int32)
    def uniform(self, shape, lo=0.0, hi=1.0):
        return jax.random.uniform(self._next(), shape, jnp.bfloat16, lo, hi)
    def permutation(self, n):
        return jax.random.permutation(self._next(), n)


kernel_name = 'concat_heads__ssm_conv_h3__compressed_kv_cla__prompt'

def setup_inputs():
    _rng = _Rng(jax.random.key(int.from_bytes(__import__("os").urandom(4), "little")))
    _w = (lambda a: (lambda t: t.astype(jnp.bfloat16) if jnp.issubdtype(t.dtype, jnp.floating) else t)(jnp.asarray(a)))
    def _A_setup():
        B, S, D = 1, 2048, 448
        ks = 4
        return {
            "q": _w((lambda *s: _rng.normal(s) * 0.05)(B, S, D)),
            "k": _w((lambda *s: _rng.normal(s) * 0.05)(B, S, D)),
            "v": _w((lambda *s: _rng.normal(s) * 0.05)(B, S, D)),
            "shift_k": _w((lambda *s: _rng.normal(s) * 0.05)(D, ks) * 0.5),
            "ssm_k": _w((lambda *s: _rng.normal(s) * 0.05)(D, S) * (1.0 / S ** 0.5)),
            "ssm_D": _w((lambda *s: _rng.normal(s) * 0.05)(D)),
        }
    _A_in = _A_setup()

    def _B_setup():
        B, H, Sq, Sk, D, M = 1, 16, 2048, 2048, 256, 448
        Dc = 4 * D
        return {
            "x": _w((lambda *s: _rng.normal(s) * 0.05)(B, Sq, M)),
            "c_kv": _w((lambda *s: _rng.normal(s) * 0.05)(B, Sk, Dc)),
            "w_q": _w((lambda *s: _rng.normal(s) * 0.05)(M, H, D) * (M ** -0.5)),
            "w_uk": _w((lambda *s: _rng.normal(s) * 0.05)(Dc, H, D) * (Dc ** -0.5)),
            "w_uv": _w((lambda *s: _rng.normal(s) * 0.05)(Dc, H, D) * (Dc ** -0.5)),
            "w_o": _w((lambda *s: _rng.normal(s) * 0.05)(H, D, M) * ((H * D) ** -0.5)),
        }
    _B_in = _B_setup()

    return {
        "A_q": _A_in["q"],
        "A_k": _A_in["k"],
        "A_v": _A_in["v"],
        "A_shift_k": _A_in["shift_k"],
        "A_ssm_k": _A_in["ssm_k"],
        "A_ssm_D": _A_in["ssm_D"],
        "B_x": _B_in["x"],
        "B_c_kv": _B_in["c_kv"],
        "B_w_q": _B_in["w_q"],
        "B_w_uk": _B_in["w_uk"],
        "B_w_uv": _B_in["w_uv"],
        "B_w_o": _B_in["w_o"],
    }

def reference(A_q, A_k, A_v, A_shift_k, A_ssm_k, A_ssm_D, B_x, B_c_kv, B_w_q, B_w_uk, B_w_uv, B_w_o):
    def _A_ref(q, k, v, shift_k, ssm_k, ssm_D):
        B, S, D = q.shape
        ks = shift_k.shape[-1]
        k_pad = jnp.pad(k, ((0, 0), (ks - 1, 0), (0, 0)))
        k_shift = jnp.zeros_like(k)
        for t in range(ks):
            k_shift = k_shift + k_pad[:, t:t + S, :] * shift_k[:, ks - 1 - t][None, None, :]
        kv = k_shift * v
        L = 2 * S
        kv_pad = jnp.pad(kv, ((0, 0), (0, S), (0, 0)))
        kf_pad = jnp.pad(ssm_k, ((0, 0), (0, S)))
        kv_f = (lambda x, axes=(-2,-1): jnp.fft.rfft2(x.astype(jnp.float32), axes=axes))(kv_pad[:, None, :, :], axes=(1, 2))
        kf_f = (lambda x, axes=(-2,-1): jnp.fft.rfft2(x.astype(jnp.float32), axes=axes))(kf_pad[:, None, :], axes=(1, 2))
        kf_f = (lambda x, *d: x.transpose(*d))(kf_f, 1, 2, 0)
        y_f = kv_f * kf_f[None, :, :, :]
        y = (lambda x, s, axes=(-2,-1): jnp.fft.irfft2(x, s=s, axes=axes).astype(jnp.bfloat16))(y_f, (1, L), axes=(1, 2))[:, 0, :S, :]
        y = y + kv * ssm_D[None, None, :]
        return q * y

    def _B_ref(x, c_kv, w_q, w_uk, w_uv, w_o):
        B, Sq, M = x.shape[0], x.shape[1], x.shape[2]
        Sk = c_kv.shape[1]
        H, D = w_q.shape[1], w_q.shape[2]
        q = jnp.einsum("bqm,mhd->bhqd", x, w_q)
        k = jnp.einsum("bkc,chd->bhkd", c_kv, w_uk)
        v = jnp.einsum("bkc,chd->bhkd", c_kv, w_uv)
        scores = jnp.einsum("bhqd,bhkd->bhqk", q, k) * (D ** -0.5)
        off = Sk - Sq
        qi = jnp.arange(Sq)[:, None]
        kj = jnp.arange(Sk)[None, :]
        cmask = kj <= (qi + off)
        scores = jnp.where(cmask[None, None], scores, -1e9)
        p = _softmax(scores, axis=-1)
        ctx = jnp.einsum("bhqk,bhkd->bhqd", p, v)
        return jnp.einsum("bhqd,hdm->bqm", ctx, w_o)

    a = _A_ref(A_q, A_k, A_v, A_shift_k, A_ssm_k, A_ssm_D)
    b = _B_ref(B_x, B_c_kv, B_w_q, B_w_uk, B_w_uv, B_w_o)
    return jnp.concatenate([a, b], axis=-1)
```

```python
import numpy as np
import jax
import jax.numpy as jnp
from jax import lax
import jax.experimental.pallas as pl
import jax.experimental.pallas.tpu as pltpu

S, DA, H, D, M, DC = 2048, 448, 16, 256, 448, 1024
C = 128
TQ = 256
NT = (((1,), (1,)), ((), ()))
F32, BF16 = jnp.float32, jnp.bfloat16


def _dft_consts():
    w = 2 * np.pi * (np.arange(C) + 0.5) / (2 * C)
    a = w[:, None] * np.arange(C)[None, :]
    fx = np.concatenate([np.cos(a), -np.sin(a)], 0)
    ak = w[:, None] * (np.arange(2 * C) - C)[None, :]
    fk = np.concatenate([np.cos(ak), -np.sin(ak)], 0)
    g = np.concatenate([np.cos(a).T, -np.sin(a).T], 1) / C
    return (np.asarray(fx, dtype=BF16), np.asarray(fk, dtype=BF16),
            np.asarray(g, dtype=BF16))


def _dot(a, b):
    return jnp.dot(a, b, preferred_element_type=F32)


def _kernel(aq, ak, akp, av, sw, sk, skp, sd, fx, fk, g,
            xt, c, wq, wuk, wuv, wo, out,
            ybuf, x, xh, kh, q_s, k_s, v_s, ctx_s, acc, bq, bk, bv, sem):
    h = pl.program_id(0)

    def cps(p):
        return [pltpu.make_async_copy(w.bitcast(jnp.uint32).at[:, p, :], b.at[p % 2],
                                      sem.at[n, p % 2])
                for n, (w, b) in enumerate(((wq, bq), (wuk, bk), (wuv, bv)))]
    pr = h // 2

    @pl.when(h == 0)
    def _():
        for cp in cps(pr):
            cp.start()

    @pl.when(h % 2 == 0)
    def _():
        @pl.when(pr + 1 < H // 2)
        def _():
            for cp in cps(pr + 1):
                cp.start()

    sh = ((1 - h % 2) * 16).astype(jnp.uint32)

    def wsel(b):
        u = (b[pr % 2] << sh) & jnp.uint32(0xFFFF0000)
        return pltpu.bitcast(u, F32).astype(BF16)

    first = h == 0
    zb = jnp.zeros((DA, C), BF16)
    kw = jnp.concatenate([jnp.where(first, zb, akp[...]), ak[...]], 1).astype(F32)
    ks = kw[:, C:] * sw[:, 0:1]
    for j in range(1, 4):
        ks = ks + pltpu.roll(kw, j, 1)[:, C:] * sw[:, j:j + 1]
    kv = ks * av[...].astype(F32)
    xh[h] = lax.dot_general(kv.astype(BF16), fx[...], NT, preferred_element_type=F32)
    kwin = jnp.concatenate([jnp.where(first, zb, skp[...]), sk[...]], 1)
    kh[h] = lax.dot_general(kwin, fk[...], NT, preferred_element_type=F32)

    R = 64
    for r in range(0, DA, R):
        def body(m, carry):
            yr, yi = carry
            kr = kh[m, r:r + R, 0:C]
            ki = kh[m, r:r + R, C:]
            xr = xh[h - m, r:r + R, 0:C]
            xi = xh[h - m, r:r + R, C:]
            return yr + (kr * xr - ki * xi), yi + (kr * xi + ki * xr)
        z = jnp.zeros((R, C), F32)
        yr, yi = lax.fori_loop(0, h + 1, body, (z, z))
        ybuf[r:r + R, 0:C] = yr.astype(BF16)
        ybuf[r:r + R, C:] = yi.astype(BF16)
    y = lax.dot_general(ybuf[...], g[...], NT, preferred_element_type=F32)
    a = aq[...].astype(F32) * (y + kv * sd[...])
    out[pl.ds(pl.multiple_of(h * C, C), C), 0:DA] = a.T.astype(out.dtype)

    @pl.when(first)
    def _():
        for t in range(0, S, TQ):
            x[t:t + TQ, :] = xt[:, t:t + TQ].astype(F32).T.astype(BF16)

    @pl.when(h % 2 == 0)
    def _():
        for cp in cps(pr):
            cp.wait()

    q_s[...] = (_dot(x[...], wsel(bq)) * (D ** -0.5)).astype(BF16)
    k_s[...] = _dot(c[...], wsel(bk)).astype(BF16)
    v_s[...] = _dot(c[...], wsel(bv)).astype(BF16)

    row = lax.broadcasted_iota(jnp.int32, (TQ, TQ), 0)
    col = lax.broadcasted_iota(jnp.int32, (TQ, TQ), 1)
    for i in range(S // TQ):
        lo = i * TQ
        q = q_s[lo:lo + TQ, :]
        sd_ = lax.dot_general(q, k_s[lo:lo + TQ, :], NT, preferred_element_type=F32)
        sd_ = jnp.where(col <= row, sd_, -1e9)
        m = jnp.max(sd_, axis=-1, keepdims=True)
        if i > 0:
            so = lax.dot_general(q, k_s[0:lo, :], NT, preferred_element_type=F32)
            m = jnp.maximum(m, jnp.max(so, axis=-1, keepdims=True))
            po = jnp.exp(so - m)
        pd = jnp.exp(sd_ - m)
        l = jnp.sum(pd, axis=-1, keepdims=True)
        o = _dot(pd.astype(BF16), v_s[lo:lo + TQ, :])
        if i > 0:
            l = l + jnp.sum(po, axis=-1, keepdims=True)
            o = o + _dot(po.astype(BF16), v_s[0:lo, :])
        ctx_s[lo:lo + TQ, :] = (o / l).astype(BF16)

    contrib = lax.dot_general(ctx_s[...], wo[...], NT, preferred_element_type=F32)

    @pl.when(first)
    def _():
        acc[...] = contrib

    @pl.when(h > 0)
    def _():
        acc[...] += contrib

    @pl.when(h == H - 1)
    def _():
        out[:, DA:DA + M] = acc[...].astype(out.dtype)


@jax.jit
def pallas_concat_heads__ssm_conv_h3__compressed_kv_cla__prompt_kernel(
    A_q, A_k, A_v, A_shift_k, A_ssm_k, A_ssm_D,
    B_x, B_c_kv, B_w_q, B_w_uk, B_w_uv, B_w_o,
):
    fx, fk, g = _dft_consts()
    fix = lambda h: (0, 0)
    one = pl.Buffered(1)
    cur = pl.BlockSpec((DA, C), lambda h: (0, h))
    prv = pl.BlockSpec((DA, C), lambda h: (0, jnp.maximum(h - 1, 0)))
    in_specs = [
        cur, cur, prv, cur, pl.BlockSpec((DA, 4), fix), cur, prv,
        pl.BlockSpec((DA, 1), fix),
        pl.BlockSpec((2 * C, C), fix), pl.BlockSpec((2 * C, 2 * C), fix),
        pl.BlockSpec((C, 2 * C), fix),
        pl.BlockSpec((M, S), fix, pipeline_mode=one),
        pl.BlockSpec((S, DC), fix, pipeline_mode=one),
        pl.BlockSpec(memory_space=pltpu.HBM),
        pl.BlockSpec(memory_space=pltpu.HBM),
        pl.BlockSpec(memory_space=pltpu.HBM),
        pl.BlockSpec((M, D), lambda h: (h, 0)),
    ]
    out = pl.pallas_call(
        _kernel,
        grid=(H,),
        in_specs=in_specs,
        out_specs=pl.BlockSpec((S, DA + M), fix),
        out_shape=jax.ShapeDtypeStruct((S, DA + M), BF16),
        scratch_shapes=[
            pltpu.VMEM((DA, 2 * C), BF16), pltpu.VMEM((S, M), BF16),
            pltpu.VMEM((H, DA, 2 * C), F32),
            pltpu.VMEM((H, DA, 2 * C), F32),
            pltpu.VMEM((S, D), BF16), pltpu.VMEM((S, D), BF16),
            pltpu.VMEM((S, D), BF16), pltpu.VMEM((S, D), BF16),
            pltpu.VMEM((S, M), F32),
            pltpu.VMEM((2, M, D), jnp.uint32), pltpu.VMEM((2, DC, D), jnp.uint32),
            pltpu.VMEM((2, DC, D), jnp.uint32), pltpu.SemaphoreType.DMA((3, 2)),
        ],
        compiler_params=pltpu.CompilerParams(
            dimension_semantics=("arbitrary",),
            vmem_limit_bytes=100 * 1024 * 1024),
    )(A_q[0].T, A_k[0].T, A_k[0].T, A_v[0].T,
      A_shift_k.astype(F32), A_ssm_k, A_ssm_k, A_ssm_D.reshape(DA, 1).astype(F32),
      fx, fk, g,
      B_x[0].T, B_c_kv[0], B_w_q, B_w_uk,
      B_w_uv, B_w_o.transpose(0, 2, 1).reshape(H * M, D))
    return out[None]


kernel = pallas_concat_heads__ssm_conv_h3__compressed_kv_cla__prompt_kernel
```

```python
import numpy as np
import jax
import jax.numpy as jnp
from jax import lax
import jax.experimental.pallas as pl
import jax.experimental.pallas.tpu as pltpu

S, DA, H, D, M, DC = 2048, 448, 16, 256, 448, 1024
C = 128
TQ = 256
NT = (((1,), (1,)), ((), ()))
F32, BF16 = jnp.float32, jnp.bfloat16


def _dft_consts():
    w = 2 * np.pi * (np.arange(C) + 0.5) / (2 * C)
    a = w[:, None] * np.arange(C)[None, :]
    fx = np.concatenate([np.cos(a), -np.sin(a)], 0)
    ak = w[:, None] * (np.arange(2 * C) - C)[None, :]
    fk = np.concatenate([np.cos(ak), -np.sin(ak)], 0)
    g = np.concatenate([np.cos(a).T, -np.sin(a).T], 1) / C
    return (np.asarray(fx, dtype=BF16), np.asarray(fk, dtype=BF16),
            np.asarray(g, dtype=BF16))


def _dot(a, b):
    return jnp.dot(a, b, preferred_element_type=F32)


def _kernel(aq, ak, akp, av, sw, sk, skp, sd, fx, fk, g,
            xt, c, wq, wuk, wuv, wo, out,
            ybuf, x, xh, kh, q_s, k_s, v_s, ctx_s, acc, bq, bk, bv, sem):
    h = pl.program_id(0)

    def cps(p):
        return [pltpu.make_async_copy(w.bitcast(jnp.uint32).at[:, p, :], b.at[p % 2],
                                      sem.at[n, p % 2])
                for n, (w, b) in enumerate(((wq, bq), (wuk, bk), (wuv, bv)))]
    pr = h // 2

    @pl.when(h == 0)
    def _():
        for cp in cps(pr):
            cp.start()

    @pl.when(h % 2 == 0)
    def _():
        @pl.when(pr + 1 < H // 2)
        def _():
            for cp in cps(pr + 1):
                cp.start()

    sh = ((1 - h % 2) * 16).astype(jnp.uint32)

    def wsel(b):
        u = (b[pr % 2] << sh) & jnp.uint32(0xFFFF0000)
        return pltpu.bitcast(u, F32).astype(BF16)

    first = h == 0
    zb = jnp.zeros((DA, C), BF16)
    kw = jnp.concatenate([jnp.where(first, zb, akp[...]), ak[...]], 1).astype(F32)
    ks = kw[:, C:] * sw[:, 0:1]
    for j in range(1, 4):
        ks = ks + pltpu.roll(kw, j, 1)[:, C:] * sw[:, j:j + 1]
    kv = ks * av[...].astype(F32)
    xh[h] = lax.dot_general(kv.astype(BF16), fx[...], NT, preferred_element_type=F32)
    kwin = jnp.concatenate([jnp.where(first, zb, skp[...]), sk[...]], 1)
    kh[h] = lax.dot_general(kwin, fk[...], NT, preferred_element_type=F32)

    R = 112
    for r in range(0, DA, R):
        def body(m, carry):
            yr, yi = carry
            kr = kh[m, r:r + R, 0:C]
            ki = kh[m, r:r + R, C:]
            xr = xh[h - m, r:r + R, 0:C]
            xi = xh[h - m, r:r + R, C:]
            return yr + (kr * xr - ki * xi), yi + (kr * xi + ki * xr)
        z = jnp.zeros((R, C), F32)
        yr, yi = lax.fori_loop(0, h + 1, body, (z, z))
        ybuf[r:r + R, 0:C] = yr.astype(BF16)
        ybuf[r:r + R, C:] = yi.astype(BF16)
    y = lax.dot_general(ybuf[...], g[...], NT, preferred_element_type=F32)
    a = aq[...].astype(F32) * (y + kv * sd[...])
    out[pl.ds(pl.multiple_of(h * C, C), C), 0:DA] = a.T.astype(out.dtype)

    @pl.when(first)
    def _():
        for t in range(0, S, TQ):
            x[t:t + TQ, :] = xt[:, t:t + TQ].astype(F32).T.astype(BF16)

    @pl.when(h % 2 == 0)
    def _():
        for cp in cps(pr):
            cp.wait()

    q_s[...] = (_dot(x[...], wsel(bq)) * (D ** -0.5)).astype(BF16)
    k_s[...] = _dot(c[...], wsel(bk)).astype(BF16)
    v_s[...] = _dot(c[...], wsel(bv)).astype(BF16)

    row = lax.broadcasted_iota(jnp.int32, (TQ, TQ), 0)
    col = lax.broadcasted_iota(jnp.int32, (TQ, TQ), 1)
    def qk(i):
        lo = i * TQ
        return lax.dot_general(q_s[lo:lo + TQ, :], k_s[0:lo + TQ, :], NT,
                               preferred_element_type=F32)

    n = S // TQ
    order = list(range(n))
    nxt = qk(order[0])
    for t, i in enumerate(order):
        lo = i * TQ
        sc = nxt
        if t + 1 < n:
            nxt = qk(order[t + 1])
        dg = jnp.where(col <= row, sc[:, lo:], -1e9)
        sc = jnp.concatenate([sc[:, :lo], dg], 1) if i else dg
        p = jnp.exp(sc - jnp.max(sc, axis=-1, keepdims=True))
        l = jnp.sum(p, axis=-1, keepdims=True)
        o = _dot(p.astype(BF16), v_s[0:lo + TQ, :])
        ctx = (o / l).astype(BF16)
        con = lax.dot_general(ctx, wo[...], NT, preferred_element_type=F32)
        acc[lo:lo + TQ, :] = jnp.where(first, 0.0, acc[lo:lo + TQ, :]) + con

    @pl.when(h == H - 1)
    def _():
        out[:, DA:DA + M] = acc[...].astype(out.dtype)


@jax.jit
def pallas_concat_heads__ssm_conv_h3__compressed_kv_cla__prompt_kernel(
    A_q, A_k, A_v, A_shift_k, A_ssm_k, A_ssm_D,
    B_x, B_c_kv, B_w_q, B_w_uk, B_w_uv, B_w_o,
):
    fx, fk, g = _dft_consts()
    fix = lambda h: (0, 0)
    one = pl.Buffered(1)
    cur = pl.BlockSpec((DA, C), lambda h: (0, h))
    prv = pl.BlockSpec((DA, C), lambda h: (0, jnp.maximum(h - 1, 0)))
    in_specs = [
        cur, cur, prv, cur, pl.BlockSpec((DA, 4), fix), cur, prv,
        pl.BlockSpec((DA, 1), fix),
        pl.BlockSpec((2 * C, C), fix), pl.BlockSpec((2 * C, 2 * C), fix),
        pl.BlockSpec((C, 2 * C), fix),
        pl.BlockSpec((M, S), fix, pipeline_mode=one),
        pl.BlockSpec((S, DC), fix, pipeline_mode=one),
        pl.BlockSpec(memory_space=pltpu.HBM),
        pl.BlockSpec(memory_space=pltpu.HBM),
        pl.BlockSpec(memory_space=pltpu.HBM),
        pl.BlockSpec((M, D), lambda h: (h, 0)),
    ]
    out = pl.pallas_call(
        _kernel,
        grid=(H,),
        in_specs=in_specs,
        out_specs=pl.BlockSpec((S, DA + M), fix),
        out_shape=jax.ShapeDtypeStruct((S, DA + M), BF16),
        scratch_shapes=[
            pltpu.VMEM((DA, 2 * C), BF16), pltpu.VMEM((S, M), BF16),
            pltpu.VMEM((H, DA, 2 * C), F32),
            pltpu.VMEM((H, DA, 2 * C), F32),
            pltpu.VMEM((S, D), BF16), pltpu.VMEM((S, D), BF16),
            pltpu.VMEM((S, D), BF16), pltpu.VMEM((S, D), BF16),
            pltpu.VMEM((S, M), F32),
            pltpu.VMEM((2, M, D), jnp.uint32), pltpu.VMEM((2, DC, D), jnp.uint32),
            pltpu.VMEM((2, DC, D), jnp.uint32), pltpu.SemaphoreType.DMA((3, 2)),
        ],
        compiler_params=pltpu.CompilerParams(
            dimension_semantics=("arbitrary",),
            vmem_limit_bytes=100 * 1024 * 1024),
    )(A_q[0].T, A_k[0].T, A_k[0].T, A_v[0].T,
      A_shift_k.astype(F32), A_ssm_k, A_ssm_k, A_ssm_D.reshape(DA, 1).astype(F32),
      fx, fk, g,
      B_x[0].T, B_c_kv[0], B_w_q, B_w_uk,
      B_w_uv, B_w_o.transpose(0, 2, 1).reshape(H * M, D))
    return out[None]


kernel = pallas_concat_heads__ssm_conv_h3__compressed_kv_cla__prompt_kernel
```
